```python
import jax
import jax.numpy as jnp

def _softmax(x, axis=-1):
    return jax.nn.softmax(x, axis=axis)
def _gelu(x):
    return jax.nn.gelu(x, approximate=True)
def _silu(x):
    return jax.nn.silu(x)
def _sigmoid(x):
    return jax.nn.sigmoid(x)
def _layernorm(x, axis=-1, eps=1e-5):
    m = jnp.mean(x, axis=axis, keepdims=True)
    v = jnp.var(x, axis=axis, keepdims=True)
    return (x - m) / jnp.sqrt(v + eps)
def _scatter_add(tgt, idx, src, axis=0):
    return tgt.at[idx].add(src)
def _segment_sum(src, seg, n):
    return jax.ops.segment_sum(src, seg, n)
class _Rng:
    def __init__(self, key):
        self._k = key
    def _next(self):
        self._k, sub = jax.random.split(self._k)
        return sub
    def normal(self, shape):
        return jax.random.normal(self._next(), shape, dtype=jnp.bfloat16)
    def randint(self, lo, hi, shape):
        return jax.random.randint(self._next(), shape, lo, hi, dtype=jnp.int32)
    def uniform(self, shape, lo=0.0, hi=1.0):
        return jax.random.uniform(self._next(), shape, jnp.bfloat16, lo, hi)
    def permutation(self, n):
        return jax.random.permutation(self._next(), n)


kernel_name = 'interleave_layers__ssm_conv_h3__mixer_s_mlp__prompt'

def setup_inputs():
    _rng = _Rng(jax.random.key(int.from_bytes(__import__("os").urandom(4), "little")))
    _w = (lambda a: (lambda t: t.astype(jnp.bfloat16) if jnp.issubdtype(t.dtype, jnp.floating) else t)(jnp.asarray(a)))
    def _A_setup():
        B, S, D = 1, 2048, 1024
        ks = 4
        return {
            "q": _w((lambda *s: _rng.normal(s) * 0.05)(B, S, D)),
            "k": _w((lambda *s: _rng.normal(s) * 0.05)(B, S, D)),
            "v": _w((lambda *s: _rng.normal(s) * 0.05)(B, S, D)),
            "shift_k": _w((lambda *s: _rng.normal(s) * 0.05)(D, ks) * 0.5),
            "ssm_k": _w((lambda *s: _rng.normal(s) * 0.05)(D, S) * (1.0 / S ** 0.5)),
            "ssm_D": _w((lambda *s: _rng.normal(s) * 0.05)(D)),
        }
    _A_in = _A_setup()

    def _B_setup():
        B, S, D, F = 1, 2048, 1024, 3584
        return {
            "x":  _w((lambda *s: _rng.normal(s) * 0.05)(B, S, D)),
            "w1": _w((lambda *s: _rng.normal(s) * 0.05)(D, D) * (D ** -0.5)),
            "w2": _w((lambda *s: _rng.normal(s) * 0.05)(D, D) * (D ** -0.5)),
            "w3": _w((lambda *s: _rng.normal(s) * 0.05)(D, F) * (D ** -0.5)),
            "w4": _w((lambda *s: _rng.normal(s) * 0.05)(F, D) * (F ** -0.5)),
        }
    _B_in = _B_setup()

    return {
        "A_q": _A_in["q"],
        "A_k": _A_in["k"],
        "A_v": _A_in["v"],
        "A_shift_k": _A_in["shift_k"],
        "A_ssm_k": _A_in["ssm_k"],
        "A_ssm_D": _A_in["ssm_D"],
        "B_x": _B_in["x"],
        "B_w1": _B_in["w1"],
        "B_w2": _B_in["w2"],
        "B_w3": _B_in["w3"],
        "B_w4": _B_in["w4"],
    }

def reference(A_q, A_k, A_v, A_shift_k, A_ssm_k, A_ssm_D, B_x, B_w1, B_w2, B_w3, B_w4):
    def _A_ref(q, k, v, shift_k, ssm_k, ssm_D):
        B, S, D = q.shape
        ks = shift_k.shape[-1]
        k_pad = jnp.pad(k, ((0, 0), (ks - 1, 0), (0, 0)))
        k_shift = jnp.zeros_like(k)
        for t in range(ks):
            k_shift = k_shift + k_pad[:, t:t + S, :] * shift_k[:, ks - 1 - t][None, None, :]
        kv = k_shift * v
        L = 2 * S
        kv_pad = jnp.pad(kv, ((0, 0), (0, S), (0, 0)))
        kf_pad = jnp.pad(ssm_k, ((0, 0), (0, S)))
        kv_f = (lambda x, axes=(-2,-1): jnp.fft.rfft2(x.astype(jnp.float32), axes=axes))(kv_pad[:, None, :, :], axes=(1, 2))
        kf_f = (lambda x, axes=(-2,-1): jnp.fft.rfft2(x.astype(jnp.float32), axes=axes))(kf_pad[:, None, :], axes=(1, 2))
        kf_f = (lambda x, *d: x.transpose(*d))(kf_f, 1, 2, 0)
        y_f = kv_f * kf_f[None, :, :, :]
        y = (lambda x, s, axes=(-2,-1): jnp.fft.irfft2(x, s=s, axes=axes).astype(jnp.bfloat16))(y_f, (1, L), axes=(1, 2))[:, 0, :S, :]
        y = y + kv * ssm_D[None, None, :]
        return q * y

    def _B_ref(x, w1, w2, w3, w4):
        B, S, D = x.shape
        h = _gelu(_layernorm(x, axis=-1) @ w1)
        c = D // 4
        g0 = jnp.pad(h[:, :, 0*c:1*c], ((0, 0), (1, 0), (0, 0)))[:, :S, :]
        g1 = jnp.pad(h[:, :, 1*c:2*c], ((0, 0), (0, 1), (0, 0)))[:, 1:, :]
        g2 = jnp.pad(h[:, :, 2*c:3*c], ((0, 0), (2, 0), (0, 0)))[:, :S, :]
        g3 = jnp.pad(h[:, :, 3*c:   ], ((0, 0), (0, 2), (0, 0)))[:, 2:, :]
        hs = jnp.concatenate([g0, g1, g2, g3], axis=-1) @ w2
        x1 = x + hs
        h2 = _gelu(_layernorm(x1, axis=-1) @ w3) @ w4
        return x1 + h2

    x = A_q
    x = x + _A_ref(_layernorm(x, axis=-1), A_k, A_v, A_shift_k, A_ssm_k, A_ssm_D)
    x = x + _B_ref(_layernorm(x, axis=-1), B_w1, B_w2, B_w3, B_w4)
    x = x + _A_ref(_layernorm(x, axis=-1), A_k, A_v, A_shift_k, A_ssm_k, A_ssm_D)
    x = x + _B_ref(_layernorm(x, axis=-1), B_w1, B_w2, B_w3, B_w4)
    return x
```

```python
import functools

import numpy as np
import jax
import jax.numpy as jnp
from jax import lax
import jax.experimental.pallas as pl
import jax.experimental.pallas.tpu as pltpu

S, D, F = 2048, 1024, 3584
N1, N2 = 128, 16
NG = 32
PAD = 8
EPS = 1e-5


def _dft_tables():
    n = S
    n1 = np.arange(N1)[None, None, :]
    n2 = np.arange(N2)[:, None, None]
    k1 = np.arange(N1)[None, :, None]
    t = N2 * n1 + n2
    s1 = np.exp(1j * np.pi * t / (2 * n) - 2j * np.pi * ((k1 * t) % n) / n)
    s1g = s1.reshape(N2, NG, 1, 4, N1)
    f1 = np.concatenate([s1g.real, s1g.imag], axis=2).reshape(N2, 2 * N1, N1)
    g1 = np.transpose(f1, (0, 2, 1)) / n
    s2 = np.exp(-2j * np.pi * np.outer(np.arange(N2), np.arange(N2)) / N2)
    blk = np.zeros((2, N2, N2, 2))
    blk[0, :, :, 0] = s2.real
    blk[0, :, :, 1] = -s2.imag
    blk[1, :, :, 0] = s2.imag
    blk[1, :, :, 1] = s2.real
    f2 = np.einsum("okni,ab->oaknib", blk, np.eye(4)).reshape(128, 128)
    g2 = f2.T
    return tuple(a.astype(np.float32) for a in (f1, g1, f2, g2))


def _ln(x):
    m = jnp.mean(x, axis=-1, keepdims=True)
    c = x - m
    v = jnp.mean(c * c, axis=-1, keepdims=True)
    return c * lax.rsqrt(v + EPS)


def _gelu(x):
    c = 0.7978845608028654
    hx = 0.5 * x
    return hx + hx * jnp.tanh(x * (c + (c * 0.044715) * (x * x)))


def _dot(a, b):
    return jnp.dot(a, b, preferred_element_type=jnp.float32)


def _kernel(q_hbm, k_hbm, v_hbm, sh_ref, h_hbm, d_ref, w1_hbm, w2_hbm, w3_hbm, w4_hbm,
            f1_hbm, g1_hbm, f2_hbm, g2_hbm, o_hbm,
            w1, w2, w3, w4, qv, y, wsem, *, CB, TM, FC):
    bf = jnp.bfloat16
    f32 = jnp.float32
    NCB = D // CB
    wcopies = [pltpu.make_async_copy(s, d, wsem.at[i]) for i, (s, d) in enumerate(
        [(q_hbm, qv), (w1_hbm, w1), (w2_hbm, w2), (w3_hbm, w3), (w4_hbm, w4)])]

    def conv(kb, vb, hb, f1, g1, f2, g2, kp, up, hp, sa, sb, sht, csem, tsem):
        def cin(c, slot):
            c0 = pl.multiple_of(c * CB, CB)
            return (pltpu.make_async_copy(k_hbm.at[:, pl.ds(c0, CB)], kb.at[slot], csem.at[slot, 0]),
                    pltpu.make_async_copy(v_hbm.at[:, pl.ds(c0, CB)], vb.at[slot], csem.at[slot, 1]),
                    pltpu.make_async_copy(h_hbm.at[pl.ds(c0, CB), :], hb.at[slot], csem.at[slot, 2]))
        for cp in cin(0, 0):
            cp.start()
        tcopies = [pltpu.make_async_copy(s, d, tsem.at[i]) for i, (s, d) in enumerate(
            [(f1_hbm, f1), (f2_hbm, f2), (g2_hbm, g2), (g1_hbm, g1)])]
        for cp in tcopies:
            cp.start()
        for cp in cin(1, 1):
            cp.start()
        for cp in wcopies:
            cp.start()
        sht[...] = sh_ref[...].astype(f32).T
        kp[0:PAD, :] = jnp.zeros((PAD, CB), f32)
        for cp in tcopies:
            cp.wait()

        def body(c, _):
            slot = c % 2
            c0 = pl.multiple_of(c * CB, CB)
            for cp in cin(c, slot):
                cp.wait()
            w = sht[:, pl.ds(c0, CB)]
            dd = d_ref[:, pl.ds(c0, CB)].astype(f32)
            kp[PAD:, :] = kb[slot].astype(f32)
            NL = CB // 128
            for l in range(NL):
                hp[l] = hb[slot, l * 128:(l + 1) * 128, :].astype(f32).T
            RB = 128
            for r in range(0, S, RB):
                ks = kp[PAD + r:PAD + r + RB, :] * w[0:1, :]
                for j in range(1, 4):
                    ks = ks + kp[PAD + r - j:PAD + r - j + RB, :] * w[j:j + 1, :]
                u = ks * vb[slot, r:r + RB, :].astype(f32)
                for l in range(NL):
                    up[l, r:r + RB, :] = u[:, l * 128:(l + 1) * 128]

            def sload(ref, n2):
                return jnp.concatenate(
                    [ref[l, pl.ds(n2, N1, stride=N2), :] for l in range(NL)], axis=1)

            @pl.when(c + 2 < NCB)
            def _():
                for cp in cin(c + 2, slot):
                    cp.start()

            for n2 in range(N2):
                sa[n2] = _dot(f1[n2], sload(up, n2).astype(bf))
                sb[n2] = _dot(f1[n2], sload(hp, n2).astype(bf))
            for g in range(NG):
                sl = slice(g * 8, g * 8 + 8)
                xa = _dot(f2[...], sa[:, sl, :].reshape(128, CB).astype(bf))
                xb = _dot(f2[...], sb[:, sl, :].reshape(128, CB).astype(bf))
                ar, ai, br, bi = xa[:64], xa[64:], xb[:64], xb[64:]
                p = jnp.concatenate([ar * br - ai * bi, ar * bi + ai * br], axis=0)
                sa[:, sl, :] = _dot(g2[...], p.astype(bf)).reshape(N2, 8, CB)
            for n2 in range(N2):
                yy = _dot(g1[n2], sa[n2].astype(bf))
                rows = pl.ds(n2, N1, stride=N2)
                yy = yy + sload(up, n2) * dd
                for l in range(NL):
                    y[c * NL + l, rows, :] = yy[:, l * 128:(l + 1) * 128]
            return 0

        lax.fori_loop(0, NCB, body, 0)

    pl.run_scoped(
        conv,
        pltpu.VMEM((2, S, CB), bf), pltpu.VMEM((2, S, CB), bf), pltpu.VMEM((2, CB, S), bf),
        pltpu.VMEM((N2, 2 * N1, N1), bf), pltpu.VMEM((N2, N1, 2 * N1), bf),
        pltpu.VMEM((128, 128), bf), pltpu.VMEM((128, 128), bf),
        pltpu.VMEM((S + PAD, CB), f32), pltpu.VMEM((CB // 128, S, 128), f32), pltpu.VMEM((CB // 128, S, 128), f32),
        pltpu.VMEM((N2, 2 * N1, CB), f32), pltpu.VMEM((N2, 2 * N1, CB), f32),
        pltpu.VMEM((4, D), f32),
        pltpu.SemaphoreType.DMA((2, 3)), pltpu.SemaphoreType.DMA((4,)))

    def mlp(xs, xn, hh, hid, ob, osem):
        NT = S // TM
        C = D // 4
        for cp in wcopies:
            cp.wait()
        hh[0:PAD, :] = jnp.zeros((PAD, D), f32)
        hh[PAD + S:, :] = jnp.zeros((PAD, D), f32)

        def p1(i, x):
            r0 = pl.multiple_of(i * TM, TM)
            rows = pl.ds(r0, TM)
            x = x + _ln(x) * jnp.concatenate([y[l, rows, :] for l in range(D // 128)], axis=1)
            n = _ln(x)
            xs[rows, :] = x
            xn[rows, :] = n
            hh[pl.ds(r0 + PAD, TM), :] = _gelu(_dot(_ln(n).astype(bf), w1[...]))

        def p2(i):
            r0 = pl.multiple_of(i * TM, TM)
            rows = pl.ds(r0, TM)
            g = jnp.concatenate([
                hh[pl.ds(r0, TM + 2 * PAD), j * C:(j + 1) * C][PAD + o:PAD + o + TM].astype(bf)
                for j, o in enumerate((-1, 1, -2, 2))], axis=1)
            x1 = xn[rows, :] + _dot(g, w2[...])
            a = _ln(x1).astype(bf)
            for f in range(0, F, FC):
                hid[:, f:f + FC] = _gelu(_dot(a, w3[:, f:f + FC])).astype(bf)
            return xs[rows, :] + x1 + _dot(hid[...], w4[...])

        def l0p1(i, _):
            p1(i, qv[pl.ds(pl.multiple_of(i * TM, TM), TM), :].astype(f32))
            return 0
        lax.fori_loop(0, NT, l0p1, 0)

        def l0p2(i, _):
            xs[pl.ds(pl.multiple_of(i * TM, TM), TM), :] = p2(i)
            return 0
        lax.fori_loop(0, NT, l0p2, 0)

        def l1p1(i, _):
            p1(i, xs[pl.ds(pl.multiple_of(i * TM, TM), TM), :])
            return 0
        lax.fori_loop(0, NT, l1p1, 0)

        def ocopy(i):
            rows = pl.ds(pl.multiple_of(i * TM, TM), TM)
            return pltpu.make_async_copy(ob.at[rows, :], o_hbm.at[rows, :], osem.at[i])

        def l1p2(i, _):
            ob[pl.ds(pl.multiple_of(i * TM, TM), TM), :] = p2(i).astype(bf)
            ocopy(i).start()
            return 0
        lax.fori_loop(0, NT, l1p2, 0)
        for i in range(NT):
            ocopy(i).wait()

    pl.run_scoped(
        mlp,
        pltpu.VMEM((S, D), f32), pltpu.VMEM((S, D), f32), pltpu.VMEM((S + 2 * PAD, D), f32),
        pltpu.VMEM((TM, F), bf), pltpu.VMEM((S, D), bf),
        pltpu.SemaphoreType.DMA((S // TM,)))


@jax.jit
def pallas_interleave_layers__ssm_conv_h3__mixer_s_mlp__prompt_kernel(
    A_q, A_k, A_v, A_shift_k, A_ssm_k, A_ssm_D, B_x, B_w1, B_w2, B_w3, B_w4,
    ):
    del B_x
    bf = jnp.bfloat16
    tables = [jnp.asarray(t, dtype=bf) for t in _dft_tables()]
    hbm = pl.BlockSpec(memory_space=pl.ANY)
    vmem = pl.BlockSpec(memory_space=pltpu.VMEM)
    out = pl.pallas_call(
        functools.partial(_kernel, CB=256, TM=512, FC=512),
        in_specs=[hbm, hbm, hbm, vmem, hbm, vmem, hbm, hbm, hbm, hbm, hbm, hbm, hbm, hbm],
        out_specs=hbm,
        out_shape=jax.ShapeDtypeStruct((S, D), bf),
        scratch_shapes=[
            pltpu.VMEM((D, D), bf), pltpu.VMEM((D, D), bf),
            pltpu.VMEM((D, F), bf), pltpu.VMEM((F, D), bf),
            pltpu.VMEM((S, D), bf), pltpu.VMEM((D // 128, S, 128), jnp.float32),
            pltpu.SemaphoreType.DMA((5,)),
        ],
        compiler_params=pltpu.CompilerParams(vmem_limit_bytes=110 * 1024 * 1024),
    )(A_q.reshape(S, D), A_k.reshape(S, D), A_v.reshape(S, D), A_shift_k, A_ssm_k,
      A_ssm_D.reshape(1, D), B_w1, B_w2, B_w3, B_w4, *tables)
    return out.reshape(1, S, D)
```

```python
import functools

import numpy as np
import jax
import jax.numpy as jnp
from jax import lax
import jax.experimental.pallas as pl
import jax.experimental.pallas.tpu as pltpu

S, D, F = 2048, 1024, 3584
N1, N2 = 128, 16
PAD = 8
WSCHED = (2, 2, 3, 4, 6)
PITCH = N2 + 1
EPS = 1e-5


def _dft_tables():
    n = S
    n1 = np.arange(N1)[None, None, :]
    n2 = np.arange(N2)[:, None, None]
    k1 = np.arange(N1)[None, :, None]
    t = N2 * n1 + n2
    s1 = np.exp(1j * np.pi * t / (2 * n) - 2j * np.pi * ((k1 * t) % n) / n)
    s1g = s1.reshape(N2, N1 // 8, 1, 8, N1)
    f1 = np.concatenate([s1g.real, s1g.imag], axis=2).reshape(N2, 2 * N1, N1)
    g1 = np.transpose(f1, (0, 2, 1)) / n
    return f1.astype(np.float32), g1.astype(np.float32)


def _fft4(x):
    (ar, ai), (br, bi), (cr, ci), (dr, di) = x
    sr, si, tr, ti = ar + cr, ai + ci, ar - cr, ai - ci
    ur, ui, vr, vi = br + dr, bi + di, br - dr, bi - di
    return [(sr + ur, si + ui), (tr + vi, ti - vr), (sr - ur, si - ui), (tr - vi, ti + vr)]


def _twiddle(z, e):
    r, i = z
    if e == 0:
        return z
    if e == 4:
        return i, -r
    h = float(np.sqrt(0.5))
    if e == 2:
        return (r + i) * h, (i - r) * h
    if e == 6:
        return (i - r) * h, (r + i) * (-h)
    c, s = float(np.cos(np.pi * e / 8)), float(np.sin(np.pi * e / 8))
    return r * c + i * s, i * c - r * s


def _fft16(x):
    cols = [_fft4([x[4 * a + b] for a in range(4)]) for b in range(4)]
    out = [None] * 16
    for ka in range(4):
        res = _fft4([_twiddle(cols[b][ka], b * ka) for b in range(4)])
        for kb in range(4):
            out[ka + 4 * kb] = res[kb]
    return out


def _ln(x):
    m = jnp.mean(x, axis=-1, keepdims=True)
    c = x - m
    v = jnp.mean(c * c, axis=-1, keepdims=True)
    return c * lax.rsqrt(v + EPS)


def _gelu(x):
    c = 0.7978845608028654
    hx = 0.5 * x
    return hx + hx * jnp.tanh(x * (c + (c * 0.044715) * (x * x)))


def _dot(a, b):
    return jnp.dot(a, b, preferred_element_type=jnp.float32)


def _kernel(q_hbm, k_hbm, v_hbm, sh_ref, h_hbm, d_ref, w1_hbm, w2_hbm, w3_hbm, w4_hbm,
            f1_hbm, g1_hbm, o_hbm,
            w1, w2, w3, w4, qv, y, wsem, *, CB, TM, FC):
    bf = jnp.bfloat16
    f32 = jnp.float32
    NCB = D // CB
    wcopies = [pltpu.make_async_copy(s, d, wsem.at[i]) for i, (s, d) in enumerate(
        [(q_hbm, qv), (w1_hbm, w1), (w2_hbm, w2), (w3_hbm, w3), (w4_hbm, w4)])]

    def conv(kb, vb, hb, f1, g1, kp, ut, ht, sa, sb, sc, yt, sht, csem, tsem):
        NL = CB // 128

        def cin(c):
            cols = pl.ds(c * CB, CB)
            return (pltpu.make_async_copy(k_hbm.at[:, cols], kb.at[c], csem.at[c, 0]),
                    pltpu.make_async_copy(v_hbm.at[:, cols], vb.at[c], csem.at[c, 1]),
                    pltpu.make_async_copy(h_hbm.at[cols, :], hb.at[c], csem.at[c, 2]))
        tcopies = [pltpu.make_async_copy(s, d, tsem.at[i]) for i, (s, d) in enumerate(
            [(f1_hbm, f1), (g1_hbm, g1)])]
        for cp in cin(0):
            cp.start()
        tcopies[0].start()
        sht[...] = sh_ref[...].astype(f32).T
        kp[0:PAD, :] = jnp.zeros((PAD, CB), f32)

        def prep(c, i):
            cols = slice(c * CB, (c + 1) * CB)
            w = sht[:, cols]
            r = pl.multiple_of(i * N1, N1)
            rp = pl.multiple_of(i * (8 * PITCH), 8)
            kc = kb[c, pl.ds(r, N1), :].astype(f32)
            win = jnp.concatenate([kp[...], kc], axis=0)
            kp[...] = kc[N1 - PAD:, :]
            ks = kc * w[0:1, :]
            for j in range(1, 4):
                ks = ks + win[PAD - j:PAD - j + N1, :] * w[j:j + 1, :]
            u = ks * vb[c, pl.ds(r, N1), :].astype(f32)
            first = (lax.broadcasted_iota(jnp.int32, (8, 128), 0) + i) == 0
            for l in range(NL):
                ls = slice(l * 128, (l + 1) * 128)
                h = hb[c, ls, pl.ds(r, N1)].astype(f32).T
                dd = d_ref[:, c * CB + l * 128:c * CB + (l + 1) * 128].astype(f32)
                for j in range(N1 // 8):
                    dst = pl.ds(rp + (j // 2) * PITCH + (j % 2) * 8, 8)
                    hj = h[8 * j:8 * j + 8, :]
                    if j == 0:
                        hj = hj + jnp.where(first, dd, 0.0)
                    ut[c % 2][l, dst, :] = u[8 * j:8 * j + 8, ls]
                    ht[c % 2][l, dst, :] = hj

        def fwd(c, i):
            rows = pl.ds(i, N1, stride=PITCH)
            for src, dst in ((ut, sa), (ht, sb)):
                x = jnp.concatenate([src[c % 2][l, rows, :] for l in range(NL)], axis=1)
                dst[c % 2][i] = _dot(f1[i], x.astype(bf))

        def mid(c, i):
            r = pl.multiple_of(i * 16, 16)
            re, im, both = pl.ds(r, 8), pl.ds(r + 8, 8), pl.ds(r, 16)
            for l in range(NL):
                ls = slice(l * 128, (l + 1) * 128)
                a = _fft16([(sa[c % 2][n, re, ls], sa[c % 2][n, im, ls]) for n in range(N2)])
                b = _fft16([(sb[c % 2][n, re, ls], sb[c % 2][n, im, ls]) for n in range(N2)])
                p = _fft16([(ar * bi + ai * br, ar * br - ai * bi)
                            for (ar, ai), (br, bi) in zip(a, b)])
                for n in range(N2):
                    sc[c % 2][n, both, ls] = jnp.concatenate(
                        [p[n][1], p[n][0]], axis=0).astype(bf)

        def inv(c, i):
            yy = _dot(g1[i], sc[c % 2][i])
            for l in range(NL):
                yt[c % 2][l, pl.ds(i, N1, stride=PITCH), :] = yy[:, l * 128:(l + 1) * 128]

        def fin(c, i):
            r = pl.multiple_of(i * N1, N1)
            rp = pl.multiple_of(i * (8 * PITCH), 8)
            for l in range(NL):
                for j in range(8):
                    y[c * NL + l, pl.ds(r + 16 * j, 16), :] = yt[c % 2][l, pl.ds(rp + j * PITCH, 16), :]

        for t in range(NCB + 4):
            if t < NCB:
                for cp in cin(t):
                    cp.wait()
                if t + 1 < NCB:
                    for cp in cin(t + 1):
                        cp.start()
                if t == 0:
                    tcopies[1].start()
                for j, cp in enumerate(wcopies):
                    if WSCHED[j] * NCB // 8 == t:
                        cp.start()
            if t in (1, 3):
                tcopies[t // 2].wait()

            def step(i, _, t=t):
                for d, fn in enumerate((prep, fwd, mid, inv, fin)):
                    if 0 <= t - d < NCB:
                        fn(t - d, i)
                return 0
            lax.fori_loop(0, N2, step, 0)
            kp[...] = jnp.zeros((PAD, CB), f32)

    pl.run_scoped(
        conv,
        pltpu.VMEM((NCB, S, CB), bf), pltpu.VMEM((NCB, S, CB), bf), pltpu.VMEM((NCB, CB, S), bf),
        pltpu.VMEM((N2, 2 * N1, N1), bf), pltpu.VMEM((N2, N1, 2 * N1), bf),
        pltpu.VMEM((PAD, CB), f32),
        [pltpu.VMEM((CB // 128, N1 * PITCH, 128), f32)] * 2,
        [pltpu.VMEM((CB // 128, N1 * PITCH, 128), f32)] * 2,
        [pltpu.VMEM((N2, 2 * N1, CB), f32)] * 2, [pltpu.VMEM((N2, 2 * N1, CB), f32)] * 2,
        [pltpu.VMEM((N2, 2 * N1, CB), bf)] * 2,
        [pltpu.VMEM((CB // 128, N1 * PITCH, 128), f32)] * 2,
        pltpu.VMEM((4, D), f32),
        pltpu.SemaphoreType.DMA((NCB, 3)), pltpu.SemaphoreType.DMA((2,)))

    def mlp(xs, xn, hh, hid, ob, osem):
        NT = S // TM
        C = D // 4
        for cp in wcopies:
            cp.wait()
        hh[0:PAD, :] = jnp.zeros((PAD, D), f32)
        hh[PAD + S:, :] = jnp.zeros((PAD, D), f32)

        def p1(i, x):
            r0 = pl.multiple_of(i * TM, TM)
            rows = pl.ds(r0, TM)
            x = x + _ln(x) * jnp.concatenate([y[l, rows, :] for l in range(D // 128)], axis=1)
            n = _ln(x)
            xs[rows, :] = x
            xn[rows, :] = n
            hh[pl.ds(r0 + PAD, TM), :] = _gelu(_dot(_ln(n).astype(bf), w1[...]))

        def p2(i):
            r0 = pl.multiple_of(i * TM, TM)
            rows = pl.ds(r0, TM)
            g = jnp.concatenate([
                hh[pl.ds(r0, TM + 2 * PAD), j * C:(j + 1) * C][PAD + o:PAD + o + TM].astype(bf)
                for j, o in enumerate((-1, 1, -2, 2))], axis=1)
            x1 = xn[rows, :] + _dot(g, w2[...])
            a = _ln(x1).astype(bf)
            for f in range(0, F, FC):
                hid[:, f:f + FC] = _gelu(_dot(a, w3[:, f:f + FC])).astype(bf)
            return xs[rows, :] + x1 + _dot(hid[...], w4[...])

        def l0p1(i, _):
            p1(i, qv[pl.ds(pl.multiple_of(i * TM, TM), TM), :].astype(f32))
            return 0
        lax.fori_loop(0, NT, l0p1, 0)

        def l0p2(i, _):
            xs[pl.ds(pl.multiple_of(i * TM, TM), TM), :] = p2(i)
            return 0
        lax.fori_loop(0, NT, l0p2, 0)

        def l1p1(i, _):
            p1(i, xs[pl.ds(pl.multiple_of(i * TM, TM), TM), :])
            return 0
        lax.fori_loop(0, NT, l1p1, 0)

        def ocopy(i):
            rows = pl.ds(pl.multiple_of(i * TM, TM), TM)
            return pltpu.make_async_copy(ob.at[rows, :], o_hbm.at[rows, :], osem.at[i])

        def l1p2(i, _):
            ob[pl.ds(pl.multiple_of(i * TM, TM), TM), :] = p2(i).astype(bf)
            ocopy(i).start()
            return 0
        lax.fori_loop(0, NT, l1p2, 0)
        for i in range(NT):
            ocopy(i).wait()

    pl.run_scoped(
        mlp,
        pltpu.VMEM((S, D), f32), pltpu.VMEM((S, D), f32), pltpu.VMEM((S + 2 * PAD, D), f32),
        pltpu.VMEM((TM, F), bf), pltpu.VMEM((S, D), bf),
        pltpu.SemaphoreType.DMA((S // TM,)))


@jax.jit
def pallas_interleave_layers__ssm_conv_h3__mixer_s_mlp__prompt_kernel(
    A_q, A_k, A_v, A_shift_k, A_ssm_k, A_ssm_D, B_x, B_w1, B_w2, B_w3, B_w4,
    ):
    del B_x
    bf = jnp.bfloat16
    tables = [jnp.asarray(t, dtype=bf) for t in _dft_tables()]
    hbm = pl.BlockSpec(memory_space=pl.ANY)
    vmem = pl.BlockSpec(memory_space=pltpu.VMEM)
    out = pl.pallas_call(
        functools.partial(_kernel, CB=128, TM=512, FC=512),
        in_specs=[hbm, hbm, hbm, vmem, hbm, vmem, hbm, hbm, hbm, hbm, hbm, hbm],
        out_specs=hbm,
        out_shape=jax.ShapeDtypeStruct((S, D), bf),
        scratch_shapes=[
            pltpu.VMEM((D, D), bf), pltpu.VMEM((D, D), bf),
            pltpu.VMEM((D, F), bf), pltpu.VMEM((F, D), bf),
            pltpu.VMEM((S, D), bf), pltpu.VMEM((D // 128, S, 128), jnp.float32),
            pltpu.SemaphoreType.DMA((5,)),
        ],
        compiler_params=pltpu.CompilerParams(vmem_limit_bytes=110 * 1024 * 1024),
    )(A_q.reshape(S, D), A_k.reshape(S, D), A_v.reshape(S, D), A_shift_k, A_ssm_k,
      A_ssm_D.reshape(1, D), B_w1, B_w2, B_w3, B_w4, *tables)
    return out.reshape(1, S, D)
```

```python
import functools

import numpy as np
import jax
import jax.numpy as jnp
from jax import lax
import jax.experimental.pallas as pl
import jax.experimental.pallas.tpu as pltpu

S, D, F = 2048, 1024, 3584
N1, N2 = 128, 16
PAD = 8
WSCHED = (2, 2, 3, 4, 6)
PITCH = N2 + 1
EPS = 1e-5


def _dft_tables():
    n = S
    n1 = np.arange(N1)[None, None, :]
    n2 = np.arange(N2)[:, None, None]
    k1 = np.arange(N1)[None, :, None]
    t = N2 * n1 + n2
    s1 = np.exp(1j * np.pi * t / (2 * n) - 2j * np.pi * ((k1 * t) % n) / n)
    s1g = s1.reshape(N2, N1 // 8, 1, 8, N1)
    f1 = np.concatenate([s1g.real, s1g.imag], axis=2).reshape(N2, 2 * N1, N1)
    g1 = np.transpose(f1, (0, 2, 1)) / n
    return f1.astype(np.float32), g1.astype(np.float32)


def _fft4(x):
    (ar, ai), (br, bi), (cr, ci), (dr, di) = x
    sr, si, tr, ti = ar + cr, ai + ci, ar - cr, ai - ci
    ur, ui, vr, vi = br + dr, bi + di, br - dr, bi - di
    return [(sr + ur, si + ui), (tr + vi, ti - vr), (sr - ur, si - ui), (tr - vi, ti + vr)]


def _twiddle(z, e):
    r, i = z
    if e == 0:
        return z
    if e == 4:
        return i, -r
    h = float(np.sqrt(0.5))
    if e == 2:
        return (r + i) * h, (i - r) * h
    if e == 6:
        return (i - r) * h, (r + i) * (-h)
    c, s = float(np.cos(np.pi * e / 8)), float(np.sin(np.pi * e / 8))
    return r * c + i * s, i * c - r * s


def _fft16(x):
    cols = [_fft4([x[4 * a + b] for a in range(4)]) for b in range(4)]
    out = [None] * 16
    for ka in range(4):
        res = _fft4([_twiddle(cols[b][ka], b * ka) for b in range(4)])
        for kb in range(4):
            out[ka + 4 * kb] = res[kb]
    return out


def _ln(x):
    m = jnp.mean(x, axis=-1, keepdims=True)
    c = x - m
    v = jnp.mean(c * c, axis=-1, keepdims=True)
    return c * lax.rsqrt(v + EPS)


def _gelu(x):
    c = 0.7978845608028654
    hx = 0.5 * x
    return hx + hx * jnp.tanh(x * (c + (c * 0.044715) * (x * x)))


def _dot(a, b):
    return jnp.dot(a, b, preferred_element_type=jnp.float32)


def _kernel(q_hbm, k_hbm, v_hbm, sh_ref, h_hbm, d_ref, w1_hbm, w2_hbm, w3_hbm, w4_hbm,
            f1_hbm, g1_hbm, o_hbm,
            w1, w2, w3, w4, qv, y, wsem, *, CB, TM, FC):
    bf = jnp.bfloat16
    f32 = jnp.float32
    NCB = D // CB
    wcopies = [pltpu.make_async_copy(s, d, wsem.at[i]) for i, (s, d) in enumerate(
        [(q_hbm, qv), (w1_hbm, w1), (w2_hbm, w2), (w3_hbm, w3), (w4_hbm, w4)])]

    def conv(kb, vb, hb, f1, g1, kp, ut, ht, sa, sb, sc, yt, sht, csem, tsem):
        NL = CB // 128

        def cin(c):
            cols = pl.ds(c * CB, CB)
            return (pltpu.make_async_copy(k_hbm.at[:, cols], kb.at[c], csem.at[c, 0]),
                    pltpu.make_async_copy(v_hbm.at[:, cols], vb.at[c], csem.at[c, 1]),
                    pltpu.make_async_copy(h_hbm.at[cols, :], hb.at[c], csem.at[c, 2]))
        tcopies = [pltpu.make_async_copy(s, d, tsem.at[i]) for i, (s, d) in enumerate(
            [(f1_hbm, f1), (g1_hbm, g1)])]
        for cp in cin(0):
            cp.start()
        tcopies[0].start()
        sht[...] = sh_ref[...].astype(f32).T
        kp[0:PAD, :] = jnp.zeros((PAD, CB), f32)

        def prep(c, i):
            cols = slice(c * CB, (c + 1) * CB)
            w = sht[:, cols]
            r = pl.multiple_of(i * N1, N1)
            rp = pl.multiple_of(i * (8 * PITCH), 8)
            kc = kb[c, pl.ds(r, N1), :].astype(f32)
            win = jnp.concatenate([kp[...], kc], axis=0)
            kp[...] = kc[N1 - PAD:, :]
            ks = kc * w[0:1, :]
            for j in range(1, 4):
                ks = ks + win[PAD - j:PAD - j + N1, :] * w[j:j + 1, :]
            u = ks * vb[c, pl.ds(r, N1), :].astype(f32)
            first = (lax.broadcasted_iota(jnp.int32, (8, 128), 0) + i) == 0
            for l in range(NL):
                ls = slice(l * 128, (l + 1) * 128)
                h = hb[c, ls, pl.ds(r, N1)].astype(f32).T
                dd = d_ref[:, c * CB + l * 128:c * CB + (l + 1) * 128].astype(f32)
                for j in range(N1 // 8):
                    dst = pl.ds(rp + (j // 2) * PITCH + (j % 2) * 8, 8)
                    hj = h[8 * j:8 * j + 8, :]
                    if j == 0:
                        hj = hj + jnp.where(first, dd, 0.0)
                    ut[c % 2][l, dst, :] = u[8 * j:8 * j + 8, ls]
                    ht[c % 2][l, dst, :] = hj

        def fwd(c, i):
            rows = pl.ds(i, N1, stride=PITCH)
            for src, dst in ((ut, sa), (ht, sb)):
                x = jnp.concatenate([src[c % 2][l, rows, :] for l in range(NL)], axis=1)
                dst[c % 2][i] = _dot(f1[i], x.astype(bf))

        def mid(c, i):
            r = pl.multiple_of(i * 16, 16)
            re, im, both = pl.ds(r, 8), pl.ds(r + 8, 8), pl.ds(r, 16)
            for l in range(NL):
                ls = slice(l * 128, (l + 1) * 128)
                a = _fft16([(sa[c % 2][n, re, ls], sa[c % 2][n, im, ls]) for n in range(N2)])
                b = _fft16([(sb[c % 2][n, re, ls], sb[c % 2][n, im, ls]) for n in range(N2)])
                p = _fft16([(ar * bi + ai * br, ar * br - ai * bi)
                            for (ar, ai), (br, bi) in zip(a, b)])
                for n in range(N2):
                    sc[c % 2][n, both, ls] = jnp.concatenate(
                        [p[n][1], p[n][0]], axis=0).astype(bf)

        def inv(c, i):
            yy = _dot(g1[i], sc[c % 2][i])
            for l in range(NL):
                yt[c % 2][l, pl.ds(i, N1, stride=PITCH), :] = yy[:, l * 128:(l + 1) * 128]

        def fin(c, i):
            r = pl.multiple_of(i * N1, N1)
            rp = pl.multiple_of(i * (8 * PITCH), 8)
            for l in range(NL):
                for j in range(8):
                    y[c * NL + l, pl.ds(r + 16 * j, 16), :] = yt[c % 2][l, pl.ds(rp + j * PITCH, 16), :]

        for t in range(NCB + 4):
            if t < NCB:
                for cp in cin(t):
                    cp.wait()
                if t + 1 < NCB:
                    for cp in cin(t + 1):
                        cp.start()
                if t == 0:
                    tcopies[1].start()
                for j, cp in enumerate(wcopies):
                    if WSCHED[j] * NCB // 8 == t:
                        cp.start()
            if t in (1, 3):
                tcopies[t // 2].wait()

            def step(i, _, t=t):
                for d, fn in enumerate((prep, fwd, mid, inv, fin)):
                    if 0 <= t - d < NCB:
                        fn(t - d, i)
                return 0
            lax.fori_loop(0, N2, step, 0)
            kp[...] = jnp.zeros((PAD, CB), f32)

    pl.run_scoped(
        conv,
        pltpu.VMEM((NCB, S, CB), bf), pltpu.VMEM((NCB, S, CB), bf), pltpu.VMEM((NCB, CB, S), bf),
        pltpu.VMEM((N2, 2 * N1, N1), bf), pltpu.VMEM((N2, N1, 2 * N1), bf),
        pltpu.VMEM((PAD, CB), f32),
        [pltpu.VMEM((CB // 128, N1 * PITCH, 128), f32)] * 2,
        [pltpu.VMEM((CB // 128, N1 * PITCH, 128), f32)] * 2,
        [pltpu.VMEM((N2, 2 * N1, CB), f32)] * 2, [pltpu.VMEM((N2, 2 * N1, CB), f32)] * 2,
        [pltpu.VMEM((N2, 2 * N1, CB), bf)] * 2,
        [pltpu.VMEM((CB // 128, N1 * PITCH, 128), f32)] * 2,
        pltpu.VMEM((4, D), f32),
        pltpu.SemaphoreType.DMA((NCB, 3)), pltpu.SemaphoreType.DMA((2,)))

    def mlp(xs, xn, hh, hid, a1, a2, ob, osem):
        NT = S // TM
        C = D // 4
        for cp in wcopies:
            cp.wait()
        hh[0:PAD, :] = jnp.zeros((PAD, D), f32)
        hh[PAD + S:, :] = jnp.zeros((PAD, D), f32)

        def row0(g):
            return pl.multiple_of((g % NT) * TM, TM)

        def gate(g):
            rows = pl.ds(row0(g), TM)
            x = jnp.where(g < NT, qv[rows, :].astype(f32), xs[rows, :]) if not isinstance(g, int) \
                else qv[rows, :].astype(f32)
            x = x + _ln(x) * jnp.concatenate([y[l, rows, :] for l in range(D // 128)], axis=1)
            n = _ln(x)
            xs[rows, :] = x + n
            xn[rows, :] = n
            a1[g % 2] = _ln(n).astype(bf)

        def tok1(g):
            hh[pl.ds(row0(g) + PAD, TM), :] = _gelu(_dot(a1[g % 2], w1[...]))

        def tok2(g):
            r0 = row0(g)
            rows = pl.ds(r0, TM)
            sh = jnp.concatenate([
                hh[pl.ds(r0, TM + 2 * PAD), j * C:(j + 1) * C][PAD + o:PAD + o + TM].astype(bf)
                for j, o in enumerate((-1, 1, -2, 2))], axis=1)
            hs = _dot(sh, w2[...])
            xs[rows, :] = xs[rows, :] + hs
            a2[g % 2] = _ln(xn[rows, :] + hs).astype(bf)

        def ocopy(i):
            rows = pl.ds(pl.multiple_of(i * TM, TM), TM)
            return pltpu.make_async_copy(ob.at[rows, :], o_hbm.at[rows, :], osem.at[i])

        def chan(g):
            rows = pl.ds(row0(g), TM)
            a = a2[g % 2]
            for f in range(0, F, FC):
                hid[:, f:f + FC] = _gelu(_dot(a, w3[:, f:f + FC])).astype(bf)
            x = xs[rows, :] + _dot(hid[...], w4[...])
            xs[rows, :] = x
            ob[rows, :] = x.astype(bf)

            @pl.when(g >= NT)
            def _():
                ocopy(g - NT).start()

        stages = ((3, tok2), (1, tok1), (0, gate), (4, chan))
        for t in range(4):
            for d, fn in stages:
                if t - d >= 0:
                    fn(t - d)

        def step(t, _):
            for d, fn in stages:
                fn(t - d)
            return 0
        lax.fori_loop(4, 2 * NT, step, 0)
        for t in range(2 * NT, 2 * NT + 3):
            for d, fn in stages:
                if t - d < 2 * NT:
                    fn(t - d)
        chan(2 * NT - 1)
        for i in range(NT):
            ocopy(i).wait()

    pl.run_scoped(
        mlp,
        pltpu.VMEM((S, D), f32), pltpu.VMEM((S, D), f32), pltpu.VMEM((S + 2 * PAD, D), f32),
        pltpu.VMEM((TM, F), bf), pltpu.VMEM((2, TM, D), bf), pltpu.VMEM((2, TM, D), bf),
        pltpu.VMEM((S, D), bf),
        pltpu.SemaphoreType.DMA((S // TM,)))


@jax.jit
def pallas_interleave_layers__ssm_conv_h3__mixer_s_mlp__prompt_kernel(
    A_q, A_k, A_v, A_shift_k, A_ssm_k, A_ssm_D, B_x, B_w1, B_w2, B_w3, B_w4,
    ):
    del B_x
    bf = jnp.bfloat16
    tables = [jnp.asarray(t, dtype=bf) for t in _dft_tables()]
    hbm = pl.BlockSpec(memory_space=pl.ANY)
    vmem = pl.BlockSpec(memory_space=pltpu.VMEM)
    out = pl.pallas_call(
        functools.partial(_kernel, CB=128, TM=128, FC=512),
        in_specs=[hbm, hbm, hbm, vmem, hbm, vmem, hbm, hbm, hbm, hbm, hbm, hbm],
        out_specs=hbm,
        out_shape=jax.ShapeDtypeStruct((S, D), bf),
        scratch_shapes=[
            pltpu.VMEM((D, D), bf), pltpu.VMEM((D, D), bf),
            pltpu.VMEM((D, F), bf), pltpu.VMEM((F, D), bf),
            pltpu.VMEM((S, D), bf), pltpu.VMEM((D // 128, S, 128), jnp.float32),
            pltpu.SemaphoreType.DMA((5,)),
        ],
        compiler_params=pltpu.CompilerParams(vmem_limit_bytes=110 * 1024 * 1024),
    )(A_q.reshape(S, D), A_k.reshape(S, D), A_v.reshape(S, D), A_shift_k, A_ssm_k,
      A_ssm_D.reshape(1, D), B_w1, B_w2, B_w3, B_w4, *tables)
    return out.reshape(1, S, D)
```

```python
import functools

import numpy as np
import jax
import jax.numpy as jnp
from jax import lax
import jax.experimental.pallas as pl
import jax.experimental.pallas.tpu as pltpu

S, D, F = 2048, 1024, 3584
N1, N2 = 128, 16
PAD = 8
LAG = 8
WSCHED = (5, 6, 7, 7, 7)
PITCH = N2 + 1
EPS = 1e-5


def _dft_tables():
    n = S
    n1 = np.arange(N1)[None, None, :]
    n2 = np.arange(N2)[:, None, None]
    k1 = np.arange(N1)[None, :, None]
    t = N2 * n1 + n2
    s1 = np.exp(1j * np.pi * t / (2 * n) - 2j * np.pi * ((k1 * t) % n) / n)
    s1g = s1.reshape(N2, N1 // 8, 1, 8, N1)
    f1 = np.concatenate([s1g.real, s1g.imag], axis=2).reshape(N2, 2 * N1, N1)
    g1 = np.transpose(f1, (0, 2, 1)) / n
    return f1.astype(np.float32), g1.astype(np.float32)


def _fft4(x):
    (ar, ai), (br, bi), (cr, ci), (dr, di) = x
    sr, si, tr, ti = ar + cr, ai + ci, ar - cr, ai - ci
    ur, ui, vr, vi = br + dr, bi + di, br - dr, bi - di
    return [(sr + ur, si + ui), (tr + vi, ti - vr), (sr - ur, si - ui), (tr - vi, ti + vr)]


def _twiddle(z, e):
    r, i = z
    if e == 0:
        return z
    if e == 4:
        return i, -r
    h = float(np.sqrt(0.5))
    if e == 2:
        return (r + i) * h, (i - r) * h
    if e == 6:
        return (i - r) * h, (r + i) * (-h)
    c, s = float(np.cos(np.pi * e / 8)), float(np.sin(np.pi * e / 8))
    return r * c + i * s, i * c - r * s


def _fft16(x):
    cols = [_fft4([x[4 * a + b] for a in range(4)]) for b in range(4)]
    out = [None] * 16
    for ka in range(4):
        res = _fft4([_twiddle(cols[b][ka], b * ka) for b in range(4)])
        for kb in range(4):
            out[ka + 4 * kb] = res[kb]
    return out


def _ln(x):
    m = jnp.mean(x, axis=-1, keepdims=True)
    c = x - m
    v = jnp.mean(c * c, axis=-1, keepdims=True)
    return c * lax.rsqrt(v + EPS)


def _gelu(x):
    c = 0.7978845608028654
    hx = 0.5 * x
    return hx + hx * jnp.tanh(x * (c + (c * 0.044715) * (x * x)))


def _dot(a, b):
    return jnp.dot(a, b, preferred_element_type=jnp.float32)


def _kernel(q_hbm, k_hbm, v_hbm, sh_ref, h_hbm, d_ref, w1_hbm, w2_hbm, w3_hbm, w4_hbm,
            f1_hbm, g1_hbm, o_hbm,
            w1, w2, w3, w4, qv, y, wsem, *, CB, TM, FC):
    bf = jnp.bfloat16
    f32 = jnp.float32
    NCB = D // CB
    wcopies = [pltpu.make_async_copy(s, d, wsem.at[i]) for i, (s, d) in enumerate(
        [(q_hbm, qv), (w1_hbm, w1), (w2_hbm, w2), (w3_hbm, w3), (w4_hbm, w4)])]

    def conv(kb, vb, hb, f1, g1, kp, ut, ht, sa, sb, sc, yt, sht, csem, tsem):
        NL = CB // 128

        def cin(c):
            cols = pl.ds(c * CB, CB)
            return (pltpu.make_async_copy(k_hbm.at[:, cols], kb.at[c], csem.at[c, 0]),
                    pltpu.make_async_copy(v_hbm.at[:, cols], vb.at[c], csem.at[c, 1]),
                    pltpu.make_async_copy(h_hbm.at[cols, :], hb.at[c], csem.at[c, 2]))
        tcopies = [pltpu.make_async_copy(s, d, tsem.at[i]) for i, (s, d) in enumerate(
            [(f1_hbm, f1), (g1_hbm, g1)])]
        for cp in cin(0):
            cp.start()
        tcopies[0].start()
        sht[0:4, :] = sh_ref[...].astype(f32)
        sht[4:5, :] = d_ref[...].astype(f32).reshape(1, D)
        kp[0:PAD, :] = jnp.zeros((PAD, CB), f32)

        def prep(c, i):
            cols = slice(c * CB, (c + 1) * CB)
            w = sht[0:4, cols]
            r = pl.multiple_of(i * N1, N1)
            rp = pl.multiple_of(i * (8 * PITCH), 8)
            kc = kb[c, pl.ds(r, N1), :].astype(f32)
            win = jnp.concatenate([kp[...], kc], axis=0)
            kp[...] = kc[N1 - PAD:, :]
            ks = kc * w[0:1, :]
            for j in range(1, 4):
                ks = ks + win[PAD - j:PAD - j + N1, :] * w[j:j + 1, :]
            u = ks * vb[c, pl.ds(r, N1), :].astype(f32)
            first = (lax.broadcasted_iota(jnp.int32, (8, 128), 0) + i) == 0
            for l in range(NL):
                ls = slice(l * 128, (l + 1) * 128)
                h = hb[c, ls, pl.ds(r, N1)].astype(f32).T
                dd = sht[4:5, c * CB + l * 128:c * CB + (l + 1) * 128]
                for j in range(N1 // 8):
                    dst = pl.ds(rp + (j // 2) * PITCH + (j % 2) * 8, 8)
                    hj = h[8 * j:8 * j + 8, :]
                    if j == 0:
                        hj = hj + jnp.where(first, dd, 0.0)
                    ut[c % 2][l, dst, :] = u[8 * j:8 * j + 8, ls]
                    ht[c % 2][l, dst, :] = hj

        def fwd(c, i):
            rows = pl.ds(i, N1, stride=PITCH)
            x = jnp.concatenate([src[c % 2][l, rows, :] for src in (ut, ht) for l in range(NL)], axis=1)
            out = _dot(f1[i], x.astype(bf))
            sa[c % 2][i] = out[:, :CB]
            sb[c % 2][i] = out[:, CB:]

        def mid(c, i):
            r = pl.multiple_of(i * 16, 16)
            re, im, both = pl.ds(r, 8), pl.ds(r + 8, 8), pl.ds(r, 16)
            for l in range(NL):
                ls = slice(l * 128, (l + 1) * 128)
                a = _fft16([(sa[c % 2][n, re, ls], sa[c % 2][n, im, ls]) for n in range(N2)])
                b = _fft16([(sb[c % 2][n, re, ls], sb[c % 2][n, im, ls]) for n in range(N2)])
                p = _fft16([(ar * bi + ai * br, ar * br - ai * bi)
                            for (ar, ai), (br, bi) in zip(a, b)])
                for n in range(N2):
                    sc[c % 2][n, both, ls] = jnp.concatenate(
                        [p[n][1], p[n][0]], axis=0).astype(bf)

        def inv(c, i):
            yy = _dot(g1[i], sc[c % 2][i])
            for l in range(NL):
                yt[c % 2][l, pl.ds(i, N1, stride=PITCH), :] = yy[:, l * 128:(l + 1) * 128]

        def fin(c, i):
            r = pl.multiple_of(i * N1, N1)
            rp = pl.multiple_of(i * (8 * PITCH), 8)
            for l in range(NL):
                for j in range(8):
                    y[c * NL + l, pl.ds(r + 16 * j, 16), :] = yt[c % 2][l, pl.ds(rp + j * PITCH, 16), :]

        for t in range(NCB + 4):
            if t < NCB:
                for cp in cin(t):
                    cp.wait()
                if t + 1 < NCB:
                    for cp in cin(t + 1):
                        cp.start()
                if t == 0:
                    tcopies[1].start()
                for j, cp in enumerate(wcopies):
                    if WSCHED[j] * NCB // 8 == t:
                        cp.start()
            if t in (1, 3):
                tcopies[t // 2].wait()

            def step(i, _, t=t):
                for d, fn in enumerate((prep, fwd, mid, inv, fin)):
                    if 0 <= t - d < NCB:
                        fn(t - d, i)
                return 0
            lax.fori_loop(0, N2, step, 0, unroll=4)
            kp[...] = jnp.zeros((PAD, CB), f32)

    pl.run_scoped(
        conv,
        pltpu.VMEM((NCB, S, CB), bf), pltpu.VMEM((NCB, S, CB), bf), pltpu.VMEM((NCB, CB, S), bf),
        pltpu.VMEM((N2, 2 * N1, N1), bf), pltpu.VMEM((N2, N1, 2 * N1), bf),
        pltpu.VMEM((PAD, CB), f32),
        [pltpu.VMEM((CB // 128, N1 * PITCH, 128), f32)] * 2,
        [pltpu.VMEM((CB // 128, N1 * PITCH, 128), f32)] * 2,
        [pltpu.VMEM((N2, 2 * N1, CB), f32)] * 2, [pltpu.VMEM((N2, 2 * N1, CB), f32)] * 2,
        [pltpu.VMEM((N2, 2 * N1, CB), bf)] * 2,
        [pltpu.VMEM((CB // 128, N1 * PITCH, 128), f32)] * 2,
        pltpu.VMEM((8, D), f32),
        pltpu.SemaphoreType.DMA((NCB, 3)), pltpu.SemaphoreType.DMA((2,)))

    def mlp(xs, xn, hh, hid, a1, a2, ob, osem):
        NT = S // TM
        C = D // 4
        for cp in wcopies[:3]:
            cp.wait()
        hh[0:PAD, :] = jnp.zeros((PAD, D), f32)
        hh[PAD + S:, :] = jnp.zeros((PAD, D), f32)

        def row0(g):
            return pl.multiple_of((g % NT) * TM, TM)

        def gate(g):
            rows = pl.ds(row0(g), TM)
            x = jnp.where(g < NT, qv[rows, :].astype(f32), xs[rows, :])
            x = x + _ln(x) * jnp.concatenate([y[l, rows, :] for l in range(D // 128)], axis=1)
            n = _ln(x)
            xs[rows, :] = x + n
            xn[rows, :] = n
            a1[g % 2] = _ln(n).astype(bf)

        def tok1(g):
            hh[pl.ds(row0(g) + PAD, TM), :] = _gelu(_dot(a1[g % 2], w1[...]))

        def tok2(g):
            r0 = row0(g)
            rows = pl.ds(r0, TM)
            sh = jnp.concatenate([
                hh[pl.ds(r0, TM + 2 * PAD), j * C:(j + 1) * C][PAD + o:PAD + o + TM].astype(bf)
                for j, o in enumerate((-1, 1, -2, 2))], axis=1)
            hs = _dot(sh, w2[...])
            xs[rows, :] = xs[rows, :] + hs
            a2[rows, :] = _ln(xn[rows, :] + hs).astype(bf)

        def ocopy(i):
            rows = pl.ds(pl.multiple_of(i * TM, TM), TM)
            return pltpu.make_async_copy(ob.at[rows, :], o_hbm.at[rows, :], osem.at[i])

        def chan(g):
            rows = pl.ds(row0(g), TM)
            a = a2[rows, :]
            for f in range(0, F, FC):
                hid[:, f:f + FC] = _gelu(_dot(a, w3[:, f:f + FC])).astype(bf)
            x = xs[rows, :] + _dot(hid[...], w4[...])
            xs[rows, :] = x
            ob[rows, :] = x.astype(bf)

            @pl.when(g >= NT)
            def _():
                ocopy(g - NT).start()

        stages = ((3, tok2), (1, tok1), (0, gate), (LAG, chan))
        cuts = sorted({d for d, _ in stages} | {d + 2 * NT for d, _ in stages})
        for lo, hi in zip(cuts, cuts[1:]):
            if lo == LAG:
                for cp in wcopies[3:]:
                    cp.wait()

            def step(t, _, lo=lo):
                for d, fn in stages:
                    if d <= lo < d + 2 * NT:
                        fn(t - d)
                return 0
            lax.fori_loop(lo, hi, step, 0)
        for i in range(NT):
            ocopy(i).wait()

    pl.run_scoped(
        mlp,
        pltpu.VMEM((S, D), f32), pltpu.VMEM((S, D), f32), pltpu.VMEM((S + 2 * PAD, D), f32),
        pltpu.VMEM((TM, F), bf), pltpu.VMEM((2, TM, D), bf), pltpu.VMEM((S, D), bf),
        pltpu.VMEM((S, D), bf),
        pltpu.SemaphoreType.DMA((S // TM,)))


@jax.jit
def pallas_interleave_layers__ssm_conv_h3__mixer_s_mlp__prompt_kernel(
    A_q, A_k, A_v, A_shift_k, A_ssm_k, A_ssm_D, B_x, B_w1, B_w2, B_w3, B_w4,
    ):
    del B_x
    bf = jnp.bfloat16
    tables = [jnp.asarray(t, dtype=bf) for t in _dft_tables()]
    hbm = pl.BlockSpec(memory_space=pl.ANY)
    vmem = pl.BlockSpec(memory_space=pltpu.VMEM)
    out = pl.pallas_call(
        functools.partial(_kernel, CB=128, TM=128, FC=512),
        in_specs=[hbm, hbm, hbm, vmem, hbm, vmem, hbm, hbm, hbm, hbm, hbm, hbm],
        out_specs=hbm,
        out_shape=jax.ShapeDtypeStruct((S, D), bf),
        scratch_shapes=[
            pltpu.VMEM((D, D), bf), pltpu.VMEM((D, D), bf),
            pltpu.VMEM((D, F), bf), pltpu.VMEM((F, D), bf),
            pltpu.VMEM((S, D), bf), pltpu.VMEM((D // 128, S, 128), jnp.float32),
            pltpu.SemaphoreType.DMA((5,)),
        ],
        compiler_params=pltpu.CompilerParams(vmem_limit_bytes=110 * 1024 * 1024),
    )(A_q.reshape(S, D), A_k.reshape(S, D), A_v.reshape(S, D), A_shift_k.T, A_ssm_k,
      A_ssm_D, B_w1, B_w2, B_w3, B_w4, *tables)
    return out.reshape(1, S, D)
```

```python
import functools

import numpy as np
import jax
import jax.numpy as jnp
from jax import lax
import jax.experimental.pallas as pl
import jax.experimental.pallas.tpu as pltpu

S, D, F = 2048, 1024, 3584
N1, N2 = 128, 16
PAD = 8
LAG = 8
WSCHED = (5, 6, 7, 7, 7)
PITCH = N2 + 1
EPS = 1e-5


def _dft_tables():
    n = S
    n1 = np.arange(N1)[None, None, :]
    n2 = np.arange(N2)[:, None, None]
    k1 = np.arange(N1)[None, :, None]
    t = N2 * n1 + n2
    s1 = np.exp(1j * np.pi * t / (2 * n) - 2j * np.pi * ((k1 * t) % n) / n)
    s1g = s1.reshape(N2, N1 // 8, 1, 8, N1)
    f1 = np.concatenate([s1g.real, s1g.imag], axis=2).reshape(N2, 2 * N1, N1)
    g1 = np.transpose(f1, (0, 2, 1)) / n
    return f1.astype(np.float32), g1.astype(np.float32)


def _fft4(x):
    (ar, ai), (br, bi), (cr, ci), (dr, di) = x
    sr, si, tr, ti = ar + cr, ai + ci, ar - cr, ai - ci
    ur, ui, vr, vi = br + dr, bi + di, br - dr, bi - di
    return [(sr + ur, si + ui), (tr + vi, ti - vr), (sr - ur, si - ui), (tr - vi, ti + vr)]


def _twiddle(z, e):
    r, i = z
    if e == 0:
        return z
    if e == 4:
        return i, -r
    h = float(np.sqrt(0.5))
    if e == 2:
        return (r + i) * h, (i - r) * h
    if e == 6:
        return (i - r) * h, (r + i) * (-h)
    c, s = float(np.cos(np.pi * e / 8)), float(np.sin(np.pi * e / 8))
    return r * c + i * s, i * c - r * s


def _fft16(x):
    cols = [_fft4([x[4 * a + b] for a in range(4)]) for b in range(4)]
    out = [None] * 16
    for ka in range(4):
        res = _fft4([_twiddle(cols[b][ka], b * ka) for b in range(4)])
        for kb in range(4):
            out[ka + 4 * kb] = res[kb]
    return out


def _ln(x):
    m = jnp.mean(x, axis=-1, keepdims=True)
    c = x - m
    v = jnp.mean(c * c, axis=-1, keepdims=True)
    return c * lax.rsqrt(v + EPS)


def _gelu(x):
    c = 0.7978845608028654
    hx = 0.5 * x
    return hx + hx * jnp.tanh(x * (c + (c * 0.044715) * (x * x)))


def _dot(a, b):
    return jnp.dot(a, b, preferred_element_type=jnp.float32)


def _kernel(q_hbm, k_hbm, v_hbm, sh_ref, h_hbm, d_ref, w1_hbm, w2_hbm, w3_hbm, w4_hbm,
            f1_hbm, g1_hbm, o_hbm,
            w1, w2, w3, w4, qv, y, wsem, *, CB, TM, FC):
    bf = jnp.bfloat16
    f32 = jnp.float32
    NCB = D // CB
    wcopies = [pltpu.make_async_copy(s, d, wsem.at[i]) for i, (s, d) in enumerate(
        [(q_hbm, qv), (w1_hbm, w1), (w2_hbm, w2), (w3_hbm, w3), (w4_hbm, w4)])]

    def conv(kb, vb, hb, f1, g1, kp, ut, ht, sa, sb, sc, yt, sht, csem, tsem):
        NL = CB // 128

        def cin(c):
            cols = pl.ds(c * CB, CB)
            return (pltpu.make_async_copy(k_hbm.at[:, cols], kb.at[c], csem.at[c, 0]),
                    pltpu.make_async_copy(v_hbm.at[:, cols], vb.at[c], csem.at[c, 1]),
                    pltpu.make_async_copy(h_hbm.at[cols, :], hb.at[c], csem.at[c, 2]))
        tcopies = [pltpu.make_async_copy(s, d, tsem.at[i]) for i, (s, d) in enumerate(
            [(f1_hbm, f1), (g1_hbm, g1)])]
        for cp in cin(0):
            cp.start()
        tcopies[0].start()
        sht[0:4, :] = sh_ref[...].astype(f32)
        sht[4:5, :] = d_ref[...].astype(f32).reshape(1, D)
        kp[0:PAD, :] = jnp.zeros((PAD, CB), f32)

        def tie(i, x, src, p):
            if src is None:
                return x
            return jnp.where(i < 0, src[8 * p:8 * p + 8, :x.shape[1]], x)

        def prep(c, i, dep):
            cols = slice(c * CB, (c + 1) * CB)
            w = sht[0:4, cols]
            r = pl.multiple_of(i * N1, N1)
            rp = pl.multiple_of(i * (8 * PITCH), 8)
            kc = kb[c, pl.ds(r, N1), :].astype(f32)
            kc = jnp.concatenate(
                [tie(i, kc[8 * j:8 * j + 8], dep, j) for j in range(N1 // 8)], axis=0)
            win = jnp.concatenate([kp[...], kc], axis=0)
            kp[...] = kc[N1 - PAD:, :]
            ks = kc * w[0:1, :]
            for j in range(1, 4):
                ks = ks + win[PAD - j:PAD - j + N1, :] * w[j:j + 1, :]
            u = ks * vb[c, pl.ds(r, N1), :].astype(f32)
            first = (lax.broadcasted_iota(jnp.int32, (8, 128), 0) + i) == 0
            for l in range(NL):
                ls = slice(l * 128, (l + 1) * 128)
                h = hb[c, ls, pl.ds(r, N1)].astype(f32).T
                dd = sht[4:5, c * CB + l * 128:c * CB + (l + 1) * 128]
                for j in range(N1 // 8):
                    dst = pl.ds(rp + (j // 2) * PITCH + (j % 2) * 8, 8)
                    hj = h[8 * j:8 * j + 8, :]
                    if j == 0:
                        hj = hj + jnp.where(first, dd, 0.0)
                    ut[c % 2][l, dst, :] = u[8 * j:8 * j + 8, ls]
                    ht[c % 2][l, dst, :] = hj

        def fwd(c, i):
            rows = pl.ds(i, N1, stride=PITCH)
            outs = []
            for src, dst in ((ut, sa), (ht, sb)):
                x = jnp.concatenate([src[c % 2][l, rows, :] for l in range(NL)], axis=1)
                outs.append(_dot(f1[i], x.astype(bf)))
                dst[c % 2][i] = outs[-1]
            return outs

        def mid(c, i, deps):
            r = pl.multiple_of(i * 16, 16)
            re, im, both = pl.ds(r, 8), pl.ds(r + 8, 8), pl.ds(r, 16)
            for l in range(NL):
                ls = slice(l * 128, (l + 1) * 128)
                a, b = [_fft16([(tie(i, src[c % 2][n, re, ls], dep, 8 * (n % 4) + 2 * (n // 4)),
                                 tie(i, src[c % 2][n, im, ls], dep, 8 * (n % 4) + 2 * (n // 4) + 1))
                                for n in range(N2)]) for src, dep in zip((sa, sb), deps)]
                p = _fft16([(ar * bi + ai * br, ar * br - ai * bi)
                            for (ar, ai), (br, bi) in zip(a, b)])
                for n in range(N2):
                    sc[c % 2][n, both, ls] = jnp.concatenate(
                        [p[n][1], p[n][0]], axis=0).astype(bf)

        def inv(c, i):
            yy = _dot(g1[i], sc[c % 2][i])
            for l in range(NL):
                yt[c % 2][l, pl.ds(i, N1, stride=PITCH), :] = yy[:, l * 128:(l + 1) * 128]
            return yy

        def fin(c, i):
            r = pl.multiple_of(i * N1, N1)
            rp = pl.multiple_of(i * (8 * PITCH), 8)
            for l in range(NL):
                for j in range(8):
                    y[c * NL + l, pl.ds(r + 16 * j, 16), :] = yt[c % 2][l, pl.ds(rp + j * PITCH, 16), :]

        for t in range(NCB + 4):
            if t < NCB:
                for cp in cin(t):
                    cp.wait()
                if t + 1 < NCB:
                    for cp in cin(t + 1):
                        cp.start()
                if t == 0:
                    tcopies[1].start()
                for j, cp in enumerate(wcopies):
                    if WSCHED[j] * NCB // 8 == t:
                        cp.start()
            if t in (1, 3):
                tcopies[t // 2].wait()

            def step(i, _, t=t):
                on = [0 <= t - d < NCB for d in range(5)]
                d_inv, d_fwd = None, (None, None)
                if on[3]:
                    d_inv = inv(t - 3, i)
                if on[0]:
                    prep(t, i, d_inv)
                if on[1]:
                    d_fwd = fwd(t - 1, i)
                if on[2]:
                    mid(t - 2, i, d_fwd)
                if on[4]:
                    fin(t - 4, i)
                return 0
            lax.fori_loop(0, N2, step, 0, unroll=8)
            kp[...] = jnp.zeros((PAD, CB), f32)

    pl.run_scoped(
        conv,
        pltpu.VMEM((NCB, S, CB), bf), pltpu.VMEM((NCB, S, CB), bf), pltpu.VMEM((NCB, CB, S), bf),
        pltpu.VMEM((N2, 2 * N1, N1), bf), pltpu.VMEM((N2, N1, 2 * N1), bf),
        pltpu.VMEM((PAD, CB), f32),
        [pltpu.VMEM((CB // 128, N1 * PITCH, 128), f32)] * 2,
        [pltpu.VMEM((CB // 128, N1 * PITCH, 128), f32)] * 2,
        [pltpu.VMEM((N2, 2 * N1, CB), f32)] * 2, [pltpu.VMEM((N2, 2 * N1, CB), f32)] * 2,
        [pltpu.VMEM((N2, 2 * N1, CB), bf)] * 2,
        [pltpu.VMEM((CB // 128, N1 * PITCH, 128), f32)] * 2,
        pltpu.VMEM((8, D), f32),
        pltpu.SemaphoreType.DMA((NCB, 3)), pltpu.SemaphoreType.DMA((2,)))

    def mlp(xs, xn, hh, hid, a1, a2, ob, osem):
        NT = S // TM
        C = D // 4
        for cp in wcopies[:3]:
            cp.wait()
        hh[0:PAD, :] = jnp.zeros((PAD, D), f32)
        hh[PAD + S:, :] = jnp.zeros((PAD, D), f32)

        def row0(g):
            return pl.multiple_of((g % NT) * TM, TM)

        def gate(g):
            rows = pl.ds(row0(g), TM)
            x = jnp.where(g < NT, qv[rows, :].astype(f32), xs[rows, :])
            x = x + _ln(x) * jnp.concatenate([y[l, rows, :] for l in range(D // 128)], axis=1)
            n = _ln(x)
            xs[rows, :] = x + n
            xn[rows, :] = n
            a1[g % 2] = _ln(n).astype(bf)

        def tok1(g):
            hh[pl.ds(row0(g) + PAD, TM), :] = _gelu(_dot(a1[g % 2], w1[...]))

        def tok2(g):
            r0 = row0(g)
            rows = pl.ds(r0, TM)
            sh = jnp.concatenate([
                hh[pl.ds(r0, TM + 2 * PAD), j * C:(j + 1) * C][PAD + o:PAD + o + TM].astype(bf)
                for j, o in enumerate((-1, 1, -2, 2))], axis=1)
            hs = _dot(sh, w2[...])
            xs[rows, :] = xs[rows, :] + hs
            a2[rows, :] = _ln(xn[rows, :] + hs).astype(bf)

        def ocopy(i):
            rows = pl.ds(pl.multiple_of(i * TM, TM), TM)
            return pltpu.make_async_copy(ob.at[rows, :], o_hbm.at[rows, :], osem.at[i])

        def chan(g):
            rows = pl.ds(row0(g), TM)
            a = a2[rows, :]
            for f in range(0, F, FC):
                hid[:, f:f + FC] = _gelu(_dot(a, w3[:, f:f + FC])).astype(bf)
            x = xs[rows, :] + _dot(hid[...], w4[...])
            xs[rows, :] = x
            ob[rows, :] = x.astype(bf)

            @pl.when(g >= NT)
            def _():
                ocopy(g - NT).start()

        stages = ((3, tok2), (1, tok1), (0, gate), (LAG, chan))
        cuts = sorted({d for d, _ in stages} | {d + 2 * NT for d, _ in stages})
        for lo, hi in zip(cuts, cuts[1:]):
            if lo == LAG:
                for cp in wcopies[3:]:
                    cp.wait()

            def step(t, _, lo=lo):
                for d, fn in stages:
                    if d <= lo < d + 2 * NT:
                        fn(t - d)
                return 0
            lax.fori_loop(lo, hi, step, 0)
        for i in range(NT):
            ocopy(i).wait()

    pl.run_scoped(
        mlp,
        pltpu.VMEM((S, D), f32), pltpu.VMEM((S, D), f32), pltpu.VMEM((S + 2 * PAD, D), f32),
        pltpu.VMEM((TM, F), bf), pltpu.VMEM((2, TM, D), bf), pltpu.VMEM((S, D), bf),
        pltpu.VMEM((S, D), bf),
        pltpu.SemaphoreType.DMA((S // TM,)))


@jax.jit
def pallas_interleave_layers__ssm_conv_h3__mixer_s_mlp__prompt_kernel(
    A_q, A_k, A_v, A_shift_k, A_ssm_k, A_ssm_D, B_x, B_w1, B_w2, B_w3, B_w4,
    ):
    del B_x
    bf = jnp.bfloat16
    tables = [jnp.asarray(t, dtype=bf) for t in _dft_tables()]
    hbm = pl.BlockSpec(memory_space=pl.ANY)
    vmem = pl.BlockSpec(memory_space=pltpu.VMEM)
    out = pl.pallas_call(
        functools.partial(_kernel, CB=128, TM=128, FC=512),
        in_specs=[hbm, hbm, hbm, vmem, hbm, vmem, hbm, hbm, hbm, hbm, hbm, hbm],
        out_specs=hbm,
        out_shape=jax.ShapeDtypeStruct((S, D), bf),
        scratch_shapes=[
            pltpu.VMEM((D, D), bf), pltpu.VMEM((D, D), bf),
            pltpu.VMEM((D, F), bf), pltpu.VMEM((F, D), bf),
            pltpu.VMEM((S, D), bf), pltpu.VMEM((D // 128, S, 128), jnp.float32),
            pltpu.SemaphoreType.DMA((5,)),
        ],
        compiler_params=pltpu.CompilerParams(vmem_limit_bytes=110 * 1024 * 1024),
    )(A_q.reshape(S, D), A_k.reshape(S, D), A_v.reshape(S, D), A_shift_k.T, A_ssm_k,
      A_ssm_D, B_w1, B_w2, B_w3, B_w4, *tables)
    return out.reshape(1, S, D)
```

```python
import functools

import numpy as np
import jax
import jax.numpy as jnp
from jax import lax
import jax.experimental.pallas as pl
import jax.experimental.pallas.tpu as pltpu

S, D, F = 2048, 1024, 3584
N1, N2 = 128, 16
PAD = 8
LAG = 8
WSCHED = (5, 6, 7, 7, 7)
PITCH = N2 + 1
EPS = 1e-5


def _dft_tables():
    n = S
    n1 = np.arange(N1)[None, None, :]
    n2 = np.arange(N2)[:, None, None]
    k1 = np.arange(N1)[None, :, None]
    t = N2 * n1 + n2
    s1 = np.exp(1j * np.pi * t / (2 * n) - 2j * np.pi * ((k1 * t) % n) / n)
    s1g = s1.reshape(N2, N1 // 8, 1, 8, N1)
    f1 = np.concatenate([s1g.real, s1g.imag], axis=2).reshape(N2, 2 * N1, N1)
    g1 = np.transpose(f1, (0, 2, 1)) / n
    return f1.astype(np.float32), g1.astype(np.float32)


def _fft4(x):
    (ar, ai), (br, bi), (cr, ci), (dr, di) = x
    sr, si, tr, ti = ar + cr, ai + ci, ar - cr, ai - ci
    ur, ui, vr, vi = br + dr, bi + di, br - dr, bi - di
    return [(sr + ur, si + ui), (tr + vi, ti - vr), (sr - ur, si - ui), (tr - vi, ti + vr)]


def _twiddle(z, e):
    r, i = z
    if e == 0:
        return z
    if e == 4:
        return i, -r
    h = float(np.sqrt(0.5))
    if e == 2:
        return (r + i) * h, (i - r) * h
    if e == 6:
        return (i - r) * h, (r + i) * (-h)
    c, s = float(np.cos(np.pi * e / 8)), float(np.sin(np.pi * e / 8))
    return r * c + i * s, i * c - r * s


def _fft16(x):
    cols = [_fft4([x[4 * a + b] for a in range(4)]) for b in range(4)]
    out = [None] * 16
    for ka in range(4):
        res = _fft4([_twiddle(cols[b][ka], b * ka) for b in range(4)])
        for kb in range(4):
            out[ka + 4 * kb] = res[kb]
    return out


def _ln(x):
    m = jnp.mean(x, axis=-1, keepdims=True)
    c = x - m
    v = jnp.mean(c * c, axis=-1, keepdims=True)
    return c * lax.rsqrt(v + EPS)


def _gelu(x):
    c = 0.7978845608028654
    hx = 0.5 * x
    return hx + hx * jnp.tanh(x * (c + (c * 0.044715) * (x * x)))


def _dot(a, b):
    return jnp.dot(a, b, preferred_element_type=jnp.float32)


def _kernel(q_hbm, k_hbm, v_hbm, sh_ref, h_hbm, d_ref, w1_hbm, w2_hbm, w3_hbm, w4_hbm,
            f1_hbm, g1_hbm, o_hbm,
            w1, w2, w3, w4, qv, y, wsem, *, CB, TM, FC):
    bf = jnp.bfloat16
    f32 = jnp.float32
    NCB = D // CB
    wcopies = [pltpu.make_async_copy(s, d, wsem.at[i]) for i, (s, d) in enumerate(
        [(q_hbm, qv), (w1_hbm, w1), (w2_hbm, w2), (w3_hbm, w3), (w4_hbm, w4)])]

    def conv(kb, vb, hb, f1, g1, kp, ut, ht, sa, sb, sc, yt, sht, csem, tsem):
        NL = CB // 128

        def cin(c):
            cols = pl.ds(c * CB, CB)
            return (pltpu.make_async_copy(k_hbm.at[:, cols], kb.at[c], csem.at[c, 0]),
                    pltpu.make_async_copy(v_hbm.at[:, cols], vb.at[c], csem.at[c, 1]),
                    pltpu.make_async_copy(h_hbm.at[cols, :], hb.at[c], csem.at[c, 2]))
        tcopies = [pltpu.make_async_copy(s, d, tsem.at[i]) for i, (s, d) in enumerate(
            [(f1_hbm, f1), (g1_hbm, g1)])]
        for cp in cin(0):
            cp.start()
        tcopies[0].start()
        sht[0:4, :] = sh_ref[...].astype(f32)
        sht[4:5, :] = d_ref[...].astype(f32).reshape(1, D)
        kp[0:PAD, :] = jnp.zeros((PAD, CB), f32)

        def tie(i, x, src, p):
            if src is None:
                return x
            return jnp.where(i < 0, src[8 * p:8 * p + 8, :x.shape[1]], x)

        def prep(c, i, dep):
            cols = slice(c * CB, (c + 1) * CB)
            w = sht[0:4, cols]
            r = pl.multiple_of(i * N1, N1)
            rp = pl.multiple_of(i * (8 * PITCH), 8)
            kc = kb[c, pl.ds(r, N1), :].astype(f32)
            kc = jnp.concatenate(
                [tie(i, kc[8 * j:8 * j + 8], dep, j) for j in range(N1 // 8)], axis=0)
            win = jnp.concatenate([kp[...], kc], axis=0)
            kp[...] = kc[N1 - PAD:, :]
            ks = kc * w[0:1, :]
            for j in range(1, 4):
                ks = ks + win[PAD - j:PAD - j + N1, :] * w[j:j + 1, :]
            u = ks * vb[c, pl.ds(r, N1), :].astype(f32)
            first = (lax.broadcasted_iota(jnp.int32, (8, 128), 0) + i) == 0
            for l in range(NL):
                ls = slice(l * 128, (l + 1) * 128)
                h = hb[c, ls, pl.ds(r, N1)].astype(f32).T
                dd = sht[4:5, c * CB + l * 128:c * CB + (l + 1) * 128]
                for j in range(N1 // 8):
                    dst = pl.ds(rp + (j // 2) * PITCH + (j % 2) * 8, 8)
                    hj = h[8 * j:8 * j + 8, :]
                    if j == 0:
                        hj = hj + jnp.where(first, dd, 0.0)
                    ut[c % 2][l, dst, :] = u[8 * j:8 * j + 8, ls]
                    ht[c % 2][l, dst, :] = hj

        def fwd(c, i):
            rows = pl.ds(i, N1, stride=PITCH)
            outs = []
            for src, dst in ((ut, sa), (ht, sb)):
                x = jnp.concatenate([src[c % 2][l, rows, :] for l in range(NL)], axis=1)
                outs.append(_dot(f1[i], x.astype(bf)))
                dst[c % 2][i] = outs[-1]
            return outs

        def mid(c, i, deps):
            r = pl.multiple_of(i * 16, 16)
            re, im, both = pl.ds(r, 8), pl.ds(r + 8, 8), pl.ds(r, 16)
            for l in range(NL):
                ls = slice(l * 128, (l + 1) * 128)
                a, b = [_fft16([(tie(i, src[c % 2][n, re, ls], dep, 8 * (n % 4) + 2 * (n // 4)),
                                 tie(i, src[c % 2][n, im, ls], dep, 8 * (n % 4) + 2 * (n // 4) + 1))
                                for n in range(N2)]) for src, dep in zip((sa, sb), deps)]
                p = _fft16([(ar * bi + ai * br, ar * br - ai * bi)
                            for (ar, ai), (br, bi) in zip(a, b)])
                for n in range(N2):
                    sc[c % 2][n, both, ls] = jnp.concatenate(
                        [p[n][1], p[n][0]], axis=0).astype(bf)

        def inv(c, i):
            yy = _dot(g1[i], sc[c % 2][i])
            for l in range(NL):
                yt[c % 2][l, pl.ds(i, N1, stride=PITCH), :] = yy[:, l * 128:(l + 1) * 128]
            return yy

        def fin(c, i):
            r = pl.multiple_of(i * N1, N1)
            rp = pl.multiple_of(i * (8 * PITCH), 8)
            for l in range(NL):
                for j in range(8):
                    y[c * NL + l, pl.ds(r + 16 * j, 16), :] = yt[c % 2][l, pl.ds(rp + j * PITCH, 16), :]

        for t in range(NCB + 4):
            if t < NCB:
                for cp in cin(t):
                    cp.wait()
                for c in ((1, 2) if t == 0 else (t + 2,)):
                    if c < NCB:
                        for cp in cin(c):
                            cp.start()
                if t == 0:
                    tcopies[1].start()
                for j, cp in enumerate(wcopies):
                    if WSCHED[j] * NCB // 8 == t:
                        cp.start()
            if t in (1, 3):
                tcopies[t // 2].wait()

            def step(i, _, t=t):
                on = [0 <= t - d < NCB for d in range(5)]
                d_inv, d_fwd = None, (None, None)
                if on[3]:
                    d_inv = inv(t - 3, i)
                if on[0]:
                    prep(t, i, d_inv)
                if on[1]:
                    d_fwd = fwd(t - 1, i)
                if on[2]:
                    mid(t - 2, i, d_fwd)
                if on[4]:
                    fin(t - 4, i)
                return 0
            lax.fori_loop(0, N2, step, 0, unroll=8)
            kp[...] = jnp.zeros((PAD, CB), f32)

    pl.run_scoped(
        conv,
        pltpu.VMEM((NCB, S, CB), bf), pltpu.VMEM((NCB, S, CB), bf), pltpu.VMEM((NCB, CB, S), bf),
        pltpu.VMEM((N2, 2 * N1, N1), bf), pltpu.VMEM((N2, N1, 2 * N1), bf),
        pltpu.VMEM((PAD, CB), f32),
        [pltpu.VMEM((CB // 128, N1 * PITCH, 128), f32)] * 2,
        [pltpu.VMEM((CB // 128, N1 * PITCH, 128), f32)] * 2,
        [pltpu.VMEM((N2, 2 * N1, CB), f32)] * 2, [pltpu.VMEM((N2, 2 * N1, CB), f32)] * 2,
        [pltpu.VMEM((N2, 2 * N1, CB), bf)] * 2,
        [pltpu.VMEM((CB // 128, N1 * PITCH, 128), f32)] * 2,
        pltpu.VMEM((8, D), f32),
        pltpu.SemaphoreType.DMA((NCB, 3)), pltpu.SemaphoreType.DMA((2,)))

    def mlp(xs, xn, hh, hid, a1, a2, ob, osem):
        NT = S // TM
        C = D // 4
        for cp in wcopies[:3]:
            cp.wait()
        hh[0:PAD, :] = jnp.zeros((PAD, D), f32)
        hh[PAD + S:, :] = jnp.zeros((PAD, D), f32)

        def row0(g):
            return pl.multiple_of((g % NT) * TM, TM)

        def gate(g):
            rows = pl.ds(row0(g), TM)
            x = jnp.where(g < NT, qv[rows, :].astype(f32), xs[rows, :])
            x = x + _ln(x) * jnp.concatenate([y[l, rows, :] for l in range(D // 128)], axis=1)
            n = _ln(x)
            xs[rows, :] = x + n
            xn[rows, :] = n
            a1[g % 2] = _ln(n).astype(bf)

        def tok1(g):
            hh[pl.ds(row0(g) + PAD, TM), :] = _gelu(_dot(a1[g % 2], w1[...]))

        def tok2(g):
            r0 = row0(g)
            rows = pl.ds(r0, TM)
            sh = jnp.concatenate([
                hh[pl.ds(r0, TM + 2 * PAD), j * C:(j + 1) * C][PAD + o:PAD + o + TM].astype(bf)
                for j, o in enumerate((-1, 1, -2, 2))], axis=1)
            hs = _dot(sh, w2[...])
            xs[rows, :] = xs[rows, :] + hs
            a2[rows, :] = _ln(xn[rows, :] + hs).astype(bf)

        def ocopy(i):
            rows = pl.ds(pl.multiple_of(i * TM, TM), TM)
            return pltpu.make_async_copy(ob.at[rows, :], o_hbm.at[rows, :], osem.at[i])

        def chan(g):
            rows = pl.ds(row0(g), TM)
            a = a2[rows, :]
            for f in range(0, F, FC):
                hid[:, f:f + FC] = _gelu(_dot(a, w3[:, f:f + FC])).astype(bf)
            x = xs[rows, :] + _dot(hid[...], w4[...])
            xs[rows, :] = x
            ob[rows, :] = x.astype(bf)

            @pl.when(g >= NT)
            def _():
                ocopy(g - NT).start()

        stages = ((3, tok2), (1, tok1), (0, gate), (LAG, chan))
        cuts = sorted({d for d, _ in stages} | {d + 2 * NT for d, _ in stages})
        for lo, hi in zip(cuts, cuts[1:]):
            if lo == LAG:
                for cp in wcopies[3:]:
                    cp.wait()

            def step(t, _, lo=lo):
                for d, fn in stages:
                    if d <= lo < d + 2 * NT:
                        fn(t - d)
                return 0
            lax.fori_loop(lo, hi, step, 0)
        for i in range(NT):
            ocopy(i).wait()

    pl.run_scoped(
        mlp,
        pltpu.VMEM((S, D), f32), pltpu.VMEM((S, D), f32), pltpu.VMEM((S + 2 * PAD, D), f32),
        pltpu.VMEM((TM, F), bf), pltpu.VMEM((2, TM, D), bf), pltpu.VMEM((S, D), bf),
        pltpu.VMEM((S, D), bf),
        pltpu.SemaphoreType.DMA((S // TM,)))


@jax.jit
def pallas_interleave_layers__ssm_conv_h3__mixer_s_mlp__prompt_kernel(
    A_q, A_k, A_v, A_shift_k, A_ssm_k, A_ssm_D, B_x, B_w1, B_w2, B_w3, B_w4,
    ):
    del B_x
    bf = jnp.bfloat16
    tables = [jnp.asarray(t, dtype=bf) for t in _dft_tables()]
    hbm = pl.BlockSpec(memory_space=pl.ANY)
    vmem = pl.BlockSpec(memory_space=pltpu.VMEM)
    out = pl.pallas_call(
        functools.partial(_kernel, CB=128, TM=128, FC=512),
        in_specs=[hbm, hbm, hbm, vmem, hbm, vmem, hbm, hbm, hbm, hbm, hbm, hbm],
        out_specs=hbm,
        out_shape=jax.ShapeDtypeStruct((S, D), bf),
        scratch_shapes=[
            pltpu.VMEM((D, D), bf), pltpu.VMEM((D, D), bf),
            pltpu.VMEM((D, F), bf), pltpu.VMEM((F, D), bf),
            pltpu.VMEM((S, D), bf), pltpu.VMEM((D // 128, S, 128), jnp.float32),
            pltpu.SemaphoreType.DMA((5,)),
        ],
        compiler_params=pltpu.CompilerParams(vmem_limit_bytes=110 * 1024 * 1024),
    )(A_q.reshape(S, D), A_k.reshape(S, D), A_v.reshape(S, D), A_shift_k.T, A_ssm_k,
      A_ssm_D, B_w1, B_w2, B_w3, B_w4, *tables)
    return out.reshape(1, S, D)
```
